```python
import jax
import jax.numpy as jnp

def _softmax(x, axis=-1):
    return jax.nn.softmax(x, axis=axis)
def _gelu(x):
    return jax.nn.gelu(x, approximate=True)
def _silu(x):
    return jax.nn.silu(x)
def _sigmoid(x):
    return jax.nn.sigmoid(x)
def _layernorm(x, axis=-1, eps=1e-5):
    m = jnp.mean(x, axis=axis, keepdims=True)
    v = jnp.var(x, axis=axis, keepdims=True)
    return (x - m) / jnp.sqrt(v + eps)
def _scatter_add(tgt, idx, src, axis=0):
    return tgt.at[idx].add(src)
def _segment_sum(src, seg, n):
    return jax.ops.segment_sum(src, seg, n)
class _Rng:
    def __init__(self, key):
        self._k = key
    def _next(self):
        self._k, sub = jax.random.split(self._k)
        return sub
    def normal(self, shape):
        return jax.random.normal(self._next(), shape, dtype=jnp.bfloat16)
    def randint(self, lo, hi, shape):
        return jax.random.randint(self._next(), shape, lo, hi, dtype=jnp.int32)
    def uniform(self, shape, lo=0.0, hi=1.0):
        return jax.random.uniform(self._next(), shape, jnp.bfloat16, lo, hi)
    def permutation(self, n):
        return jax.random.permutation(self._next(), n)


kernel_name = 'sequential_preLN__spectral_gfnet__swiglu_ffn__prompt'

def _fwd_setup_inputs():
    _rng = _Rng(jax.random.key(int.from_bytes(__import__("os").urandom(4), "little")))
    _w = (lambda a: (lambda t: t.astype(jnp.bfloat16) if jnp.issubdtype(t.dtype, jnp.floating) else t)(jnp.asarray(a)))
    def _A_setup():
        B, S, D = 1, 2048, 576
        Df = D // 2 + 1
        return {
            "x": _w((lambda *s: _rng.normal(s) * 0.05)(B, S, D)),
            "w_r": _w((lambda *s: _rng.normal(s) * 0.05)(S, Df) * 0.02),
            "w_i": _w((lambda *s: _rng.normal(s) * 0.05)(S, Df) * 0.02),
        }
    _A_in = _A_setup()

    def _B_setup():
        B, S, D, F = 1, 2048, 576, 4608
        return {
            "x": _w((lambda *s: _rng.normal(s) * 0.05)(B, S, D)),
            "w_gate": _w((lambda *s: _rng.normal(s) * 0.05)(D, F)),
            "w_up": _w((lambda *s: _rng.normal(s) * 0.05)(D, F)),
            "w_down": _w((lambda *s: _rng.normal(s) * 0.05)(F, D)),
        }
    _B_in = _B_setup()

    return {
        "A_x": _A_in["x"],
        "A_w_r": _A_in["w_r"],
        "A_w_i": _A_in["w_i"],
        "B_x": _B_in["x"],
        "B_w_gate": _B_in["w_gate"],
        "B_w_up": _B_in["w_up"],
        "B_w_down": _B_in["w_down"],
    }

def _fwd_reference(A_x, A_w_r, A_w_i, B_x, B_w_gate, B_w_up, B_w_down):
    def _A_ref(x, w_r, w_i):
        B, S, D = x.shape
        X = (lambda x, axes=(-2,-1): jnp.fft.rfft2(x.astype(jnp.float32), axes=axes))(x, axes=(-2, -1))
        W = w_r + 1j * w_i
        X = X * W
        y = (lambda x, s, axes=(-2,-1): jnp.fft.irfft2(x, s=s, axes=axes).astype(jnp.bfloat16))(X, (S, D), axes=(-2, -1))
        return y

    def _B_ref(x, w_gate, w_up, w_down):
        g = _silu(x @ w_gate)
        u = x @ w_up
        return (g * u) @ w_down

    x = A_x
    h = x + _A_ref(_layernorm(x, axis=-1), A_w_r, A_w_i)
    h2 = h + _B_ref(_layernorm(h, axis=-1), B_w_gate, B_w_up, B_w_down)
    return h2


def setup_inputs():
    _inp = _fwd_setup_inputs()
    _gk = jax.random.fold_in(jax.random.key(int.from_bytes(__import__("os").urandom(4), "little")), 2**31 - 1)
    _shapes = [[1, 2048, 576]]
    _dtypes = ['bfloat16']
    _gks = jax.random.split(_gk, len(_shapes))
    _gs = [jax.random.normal(k, s, dtype=jnp.dtype(d)) * 0.05 for k, s, d in zip(_gks, _shapes, _dtypes)]
    _inp["grad_out"] = _gs[0]
    return _inp

def reference(A_x, A_w_r, A_w_i, B_w_gate, B_w_up, B_w_down, B_x, grad_out):
    _const = dict(B_x=B_x)
    def _f(*_d):
        return _fwd_reference(**{'A_x': _d[0], 'A_w_r': _d[1], 'A_w_i': _d[2], 'B_w_gate': _d[3], 'B_w_up': _d[4], 'B_w_down': _d[5], **_const})
    _out, _vjp = jax.vjp(_f, A_x, A_w_r, A_w_i, B_w_gate, B_w_up, B_w_down)
    _grads = _vjp(grad_out)
    _out0 = jnp.asarray(_out)
    return (_out0, *[jnp.asarray(_g) for _g in _grads])
```

```python
from functools import partial

import numpy as np
import jax
import jax.numpy as jnp
from jax import lax
import jax.experimental.pallas as pl
import jax.experimental.pallas.tpu as pltpu

S, D, F = 2048, 576, 4608
DF = D // 2 + 1
LP = 304
NT = S // 128
FT = 256
ST = 1024
H2, W2, D2 = ST // 2, FT // 2, D // 2
NF = F // FT
EPS = 1e-5
bf16, f32 = jnp.bfloat16, jnp.float32


CLASSES = [(l0, 32 * n, 32) for n, l0 in enumerate((1, 8, 2, 7, 3, 6, 4, 5, 0))]
_B = np.arange(1, 5)
COS9 = np.cos(2 * np.pi * np.outer(_B, _B) / 9)
SIN9 = np.sin(2 * np.pi * np.outer(_B, _B) / 9)


def _consts():
    d2 = np.arange(64)[None, :]

    def block(l, sign):
        a = 2.0 * np.pi * ((l[:, None] * d2) % D) / D
        re = np.concatenate([np.cos(a), sign * np.sin(a)], axis=1)
        im = np.concatenate([-np.sin(a), sign * np.cos(a)], axis=1)
        return re, im
    cd = np.zeros((5, 128, 128))
    ms = np.full((5, 128), 2.0 / (S * D))
    for r in range(1, 5):
        (ra, ia), (rb, ib) = block(r + 9 * np.arange(32), -1), block(9 - r + 9 * np.arange(32), 1)
        cd[r - 1] = np.concatenate([ra, rb, ia, ib])
    r0, i0 = block(9 * np.arange(33), 0)
    cd[4, 0:33], cd[4, 49:80] = r0, i0[1:32]
    ms[4, 0] = ms[4, 32] = 1.0 / (S * D)
    ci = (cd * ms[:, :, None]).transpose(0, 2, 1)
    q = np.arange(128)
    s2 = np.arange(128)[:, None]
    bs = np.zeros((NT, 256, 256))
    for k1 in range(NT):
        tile = (q - k1) % 16
        k = 128 * tile + (q - tile) % 128
        a = 2.0 * np.pi * ((s2 * k[None, :]) % S) / S
        mr, mi = np.cos(a), -np.sin(a)
        bs[k1] = np.block([[mr, mi], [-mi, mr]])
    t = lambda v: np.asarray(v, np.float32).astype(bf16)
    return t(cd), t(ci), t(bs)


_CD, _CI, _BS = _consts()


def _nn(a, b):
    return lax.dot_general(a, b, (((1,), (0,)), ((), ())), preferred_element_type=f32)


def _nt(a, b):
    return lax.dot_general(a, b, (((1,), (1,)), ((), ())), preferred_element_type=f32)


def _tw(re, im, p, sign):
    p = p % 16
    if p == 0:
        return re, im
    if p == 4:
        return (-im, re) if sign > 0 else (im, -re)
    if p == 8:
        return -re, -im
    c = float(np.cos(2 * np.pi * p / 16))
    s = float(sign * np.sin(2 * np.pi * p / 16))
    if p % 2 == 0:
        q = s / c
        if q > 0:
            return (re - im) * c, (re + im) * c
        return (re + im) * c, (im - re) * c
    return re * c - im * s, re * s + im * c


def _fft4(v, sign):
    (ar, ai), (br, bi), (cr, ci), (dr, di) = v
    pr, pi_, qr, qi = ar + cr, ai + ci, ar - cr, ai - ci
    sr, si, tr, ti = br + dr, bi + di, br - dr, bi - di
    o1, o3 = (qr - ti, qi + tr), (qr + ti, qi - tr)
    if sign < 0:
        o1, o3 = o3, o1
    return [(pr + sr, pi_ + si), o1, (pr - sr, pi_ - si), o3]


def _fft16(v, sign):
    cols = [_fft4([v[4 * a + b] for a in range(4)], sign) for b in range(4)]
    out = [None] * 16
    for c in range(4):
        r = _fft4([_tw(*cols[b][c], b * c, sign) for b in range(4)], sign)
        for e in range(4):
            out[c + 4 * e] = r[e]
    return out


def _lin(coef, vals):
    out = None
    for c, v in zip(coef, vals):
        if abs(c) > 1e-12:
            out = float(c) * v if out is None else out + float(c) * v
    return out


def _radix9(x):
    sm = [x[b] + x[9 - b] for b in range(1, 5)]
    df = [x[b] - x[9 - b] for b in range(1, 5)]
    out = []
    for r in range(4):
        out += [x[0] + _lin(COS9[r], sm), _lin(SIN9[r], df)]
    return out + [x[0] + (sm[0] + sm[1]) + (sm[2] + sm[3])]


def _radix9_t(v):
    re, im, dc = v[0:8:2], v[1:8:2], v[8]
    sm = [dc + _lin(COS9[b], re) for b in range(4)]
    df = [_lin(SIN9[b], im) for b in range(4)]
    return ([dc + (re[0] + re[1]) + (re[2] + re[3])] + [sm[b] + df[b] for b in range(4)]
            + [sm[b] - df[b] for b in (3, 2, 1, 0)])


def _barrel(t, sign):
    lane = lax.broadcasted_iota(jnp.int32, t[0].shape, 1)
    for i in range(4):
        hi = (lane & (1 << i)) != 0
        t = [jnp.where(hi, t[(p + sign * (1 << i)) % 16], t[p]) for p in range(16)]
    return t


def _to_spectral_order(t):
    r = [pltpu.roll(v, n, 1) if n else v for n, v in enumerate(t)]
    return _barrel([r[-m % 16] for m in range(16)], -1)


def _to_natural_order(t):
    r = _barrel(t, +1)
    return [pltpu.roll(r[-n % 16], 128 - n, 1) if n else r[0] for n in range(16)]


def _lhs7(a11, a12, a21, a22):
    return [a11 + a22, a21 + a22, a11, a22, a11 + a12, a21 - a11, a12 - a22]


def _rhs7(b11, b12, b21, b22):
    return [b11 + b22, b11, b12 - b22, b21 - b11, b22, b11 + b12, b21 + b22]


def _sum7(m):
    return (m[0] + m[3] - m[4] + m[6], m[2] + m[4], m[1] + m[3], m[0] - m[1] + m[2] + m[5])


def _lhs7t(a11, a12, a21, a22):
    return [a11 - a22, a21 - a22, a12 - a22, a11 - a21, a11 - a12, a22, a11]


def _sum7t(n):
    return (n[0] + n[5] - n[4] + n[2], n[6] - n[4], n[1] + n[5], n[1] - n[0] + n[6] - n[3])


def _quad(v, r, c):
    return v[:r, :c], v[:r, c:2 * c], v[r:2 * r, :c], v[r:2 * r, c:2 * c]


def _tile(t):
    return slice(128 * t, 128 * (t + 1))


def _ln(v):
    c = v - jnp.mean(v, axis=0, keepdims=True)
    r = lax.rsqrt(jnp.mean(c * c, axis=0, keepdims=True) + EPS)
    return c * r, r


def _ln_bwd(n, r, g):
    return r * (g - jnp.mean(g, axis=0, keepdims=True)
                - n * jnp.mean(g * n, axis=0, keepdims=True))


def _kernel(xT_h, doT_h, wrT_h, wiT_h, cd_h, ci_h, bs_h, wg_h, wu_h, wdT_h,
            outT_h, dxT_h, dwrT_h, dwiT_h, dwg_h, dwu_h, dwdT_h,
            xT, doT, wv, cd, ci, bs, wts, gws, oT, dwv,
            xnT, r1, hnT, r2, ub, yv, z, zb, xs, wp, dhT, big, tok, zs, accO, accG, gacc,
            hA, dA, hTA, dTA, wB, wA,
            sem_in, sem_w, sem_g, sem_o):
    def cols(i, n):
        return pl.ds(pl.multiple_of(i * n, n), n)

    def in_copy(k):
        src, dst = ((xT_h, xT), (cd_h, cd), (wrT_h, wv.at[0]), (wiT_h, wv.at[1]),
                    (doT_h, doT), (bs_h, bs), (ci_h, ci))[k]
        return pltpu.make_async_copy(src, dst, sem_in.at[k])

    def w_copy(k, f):
        return pltpu.make_async_copy((wg_h, wu_h, wdT_h)[k].at[:, cols(f, FT)],
                                     wts.at[k, f % 2], sem_w.at[k, f % 2])

    def g_copy(k, f):
        return pltpu.make_async_copy(gws.at[k, f % 2], (dwg_h, dwu_h, dwdT_h)[k].at[:, cols(f, FT)],
                                     sem_g.at[k, f % 2])

    def o_copy(k):
        src, dst = ((oT.at[0], outT_h), (dwv.at[0], dwrT_h), (dwv.at[1], dwiT_h))[k]
        return pltpu.make_async_copy(src, dst, sem_o.at[k])

    def dx_copy(n):
        return pltpu.make_async_copy(oT.at[1, :, cols(n, 256)], dxT_h.at[:, cols(n, 256)],
                                     sem_o.at[3 + n])

    in_copy(0).start()
    in_copy(1).start()

    def loop(n, fn):
        lax.fori_loop(0, n, lambda i, c: (fn(i), c)[1], 0)

    def rws(start, n):
        return pl.ds(start if isinstance(start, int) else pl.multiple_of(start, 16), n)

    def rows(i):
        return cols(i, 16)

    def rows_im(i):
        return pl.ds(pl.multiple_of(LP + i * 16, 16), 16)

    def butterflies(v, c):
        u = _radix9([v[64 * b:64 * (b + 1)] for b in range(9)])
        for b in range(9):
            ub[64 * b:64 * (b + 1), c] = u[b].astype(bf16)

    def unbutterfly(c):
        return jnp.concatenate(_radix9_t([yv[64 * b:64 * (b + 1), c] for b in range(9)]), axis=0)

    def spectral(filt, side=None, side_last=None):
        for r in range(4):
            v = _nn(cd[r], ub[128 * r:128 * (r + 1), :])
            z[64 * r:64 * (r + 1), :] = v[0:64]
            z[LP + 64 * r:LP + 64 * (r + 1), :] = v[64:128]
        v = _nn(cd[4, 0:96, 0:64], ub[512:576, :])
        z[256:LP, :] = v[0:48]
        z[LP + 256:2 * LP, :] = v[48:96]

        def fft16(i, sign):
            v = [(z[rows(i), _tile(t)], z[rows_im(i), _tile(t)]) for t in range(NT)]
            o = _fft16(v, sign)
            for t in range(NT):
                zb[t, rows(i), 0:128] = o[t][0].astype(bf16)
                zb[t, rows(i), 128:256] = o[t][1].astype(bf16)
        if side is None:
            loop(LP // 16, partial(fft16, sign=-1))
        else:
            loop(LP // 16 - 1, lambda i: (fft16(i, -1), side(i)))
            fft16(LP // 16 - 1, -1)
            side(None)

        def sstage(j):
            for t in [4 * j + n for n in range(4)]:
                v = _nn(zb[t], bs[t])
                yr, yi = filt(t, v[:, 0:128], v[:, 128:256])
                v = _nt(jnp.concatenate([yr, yi], axis=1).astype(bf16), bs[t])
                z[0:LP, cols(t, 128)] = v[:, 0:128]
                z[LP:2 * LP, cols(t, 128)] = v[:, 128:256]
        loop(NT // 4, sstage)
        if side_last is None:
            loop(LP // 16, partial(fft16, sign=1))
        else:
            loop(LP // 16 - 1, lambda i: (fft16(i, 1), side_last(i)))
            fft16(LP // 16 - 1, 1)
            side_last(None)

        def istage(j):
            for r, (a, b) in enumerate([(64 * n, 64 * n + 64) for n in range(4)] + [(256, LP)]):
                rhs = jnp.concatenate(
                    [jnp.concatenate([zb[4 * j + n, a:b, 0:128], zb[4 * j + n, a:b, 128:256]], axis=0)
                     for n in range(4)], axis=1)
                m = 128 if r < 4 else 64
                yv[128 * r:128 * r + m, cols(j, 512)] = _nn(ci[r, 0:m, 0:2 * (b - a)], rhs)
        loop(NT // 4, istage)

    def weights(k, t):
        return jnp.concatenate([wp[k, t, pl.ds(l0, n, stride=9), :] for l0, _, n in CLASSES]
                               + [wp[k, t, DF - 1:LP, :]], axis=0)

    def pair(n):
        s_, t = n // 4, n % 4
        return s_, cols(t, 128), cols(s_ * 8 + t, 128), cols(s_ * 8 + 4 + t, 128)

    def clear(n):
        s_, c, _, _ = pair(n)
        for i in range(7):
            accG[s_, i, :, c] = jnp.zeros((D2, 128), f32)
            if i in (0, 4, 5):
                accO[s_, i, :, c] = jnp.zeros((D2, 128), f32)
    loop(8, clear)
    in_copy(0).wait()
    for k in (2, 3, 5):
        in_copy(k).start()

    def ln1(t):
        c = cols(t, 128)
        n, r = _ln(xT[:, c].astype(f32))
        xnT[:, c] = n.astype(bf16)
        r1[:, c] = r
        butterflies(n, c)
    loop(NT, ln1)
    for k in (1, 2, 3, 5):
        in_copy(k).wait()
    in_copy(4).start()
    in_copy(6).start()
    for f in range(2):
        for k in range(3):
            w_copy(k, f).start()

    def wperm(i):
        for k in range(2):
            if i is None:
                last = jnp.broadcast_to(wv[k, DF - 1:DF, :].astype(f32), (16, S))
                first_row = lax.broadcasted_iota(jnp.int32, (16, S), 0) == 0
                v, rr = jnp.where(first_row, last, 0.0).astype(bf16), slice(DF - 1, LP)
            else:
                v, rr = wv[k, rows(i), :], rows(i)
            o = _to_spectral_order([pltpu.bitcast(v[:, _tile(t)], jnp.uint32) for t in range(NT)])
            for t in range(NT):
                wp[k, t, rr, :] = pltpu.bitcast(o[t], bf16).astype(f32)
        if i is None:
            in_copy(6).wait()

    def filt(t, xr, xi):
        row = lax.broadcasted_iota(jnp.int32, (LP, 128), 0)
        sc = jnp.where((row == 256) | (row == 288), 1.0 / (S * D), 2.0 / (S * D)).astype(f32)
        wr, wi = weights(0, t), weights(1, t)
        xs[0, t] = xr * sc
        xs[1, t] = xi * sc
        return xr * wr - xi * wi, xr * wi + xi * wr
    spectral(filt, side=wperm)
    in_copy(4).wait()

    KS = (256, 256, 320, 320, 256, 320, 320)

    def operands(s_, c, u, v, lhs, lhs_t):
        uf, vf = u.astype(f32), v.astype(f32)
        for i, o in enumerate(_lhs7(uf[:D2], vf[:D2], uf[D2:], vf[D2:])):
            lhs_t[s_, i, :, c] = o.astype(bf16)
        uf, vf = u.T.astype(f32), v.T.astype(f32)
        for i, o in enumerate(_lhs7(uf[:, :256], uf[:, 256:512], vf[:, :256], vf[:, 256:512])):
            lhs[s_, i, c, 0:256] = o.astype(bf16)
        t1, t2 = uf[:, 512:], vf[:, 512:]
        for i, o in ((2, t1), (3, t2), (5, t2 - t1), (6, t1 - t2)):
            lhs[s_, i, c, 256:320] = o.astype(bf16)

    def ln2(n):
        s_, c, c1, c2 = pair(n)
        h, nb = [], []
        for cc in (c1, c2):
            h.append(unbutterfly(cc) + xT[:, cc].astype(f32))
            v, r = _ln(h[-1])
            nb.append(v.astype(bf16))
            hnT[:, cc] = nb[-1]
            r2[:, cc] = r
        accO[s_, 2, :, c] = h[0][:D2]
        accO[s_, 6, :, c] = h[1][:D2]
        accO[s_, 1, :, c] = h[0][D2:]
        accO[s_, 3, :, c] = h[1][:D2] + h[0][D2:] - h[1][D2:]
        operands(s_, c, nb[0], nb[1], hA, hTA)
        operands(s_, c, doT[:, c1], doT[:, c2], dA, dTA)
    loop(8, ln2)

    tok[...] = jnp.zeros_like(tok)
    for n in range(4):
        zs[n] = 0

    def gated(v, z0):
        zero = tok[pl.ds(pl.multiple_of(z0, 8), 8), :]
        u = pltpu.bitcast(v, jnp.uint32)
        return pltpu.bitcast(u | jnp.tile(zero, (u.shape[0] // 8, u.shape[1] // 128)), v.dtype)

    def prep(f, half, z0, k):
        c = slice(k * W2, (k + 1) * W2)

        def blocks(r0, r1_, n):
            top = gated(wts[k, f % 2, rws(r0, n), :], z0).astype(f32)
            bot = gated(wts[k, f % 2, rws(r1_, n), :], z0).astype(f32)
            return top[:, :W2], top[:, W2:], bot[:, :W2], bot[:, W2:]

        def fwd(r):
            r = half * 128 + r
            return [(wB, (f % 2, i, rws(r, 32), c), o.astype(bf16))
                    for i, o in enumerate(_rhs7(*blocks(r, 256 + r, 32)))]

        def tail():
            v = wts[k, f % 2, rws(512 + half * 32, 32), :]
            return [(wB, (f % 2, i, rws(256 + half * 32, 32), c), v[:, n * W2:(n + 1) * W2])
                    for i, n in ((2, 1), (3, 0), (5, 1), (6, 0))]

        def bwd(r):
            r = half * (D2 // 2) + r
            return [(wA, (f % 3, i, rws(r, 48), c), o.astype(bf16))
                    for i, o in enumerate(_lhs7t(*blocks(r, D2 + r, 48)))]
        return ([partial(fwd, r) for r in range(0, 128, 32)] + [tail]
                + [partial(bwd, r) for r in range(0, D2 // 2, 48)])

    def finish_w(f, half, z0, k):
        def piece(r):
            r = half * (D2 // 2) + r
            cq = _sum7([gated(gacc[f % 2, i, rws(r, 48), k * W2:(k + 1) * W2], z0)
                        for i in range(7)])
            return [(gws, (k, f % 2, rws((n // 2) * D2 + r, 48),
                           slice((n % 2) * W2, (n % 2 + 1) * W2)), cq[n].astype(bf16))
                    for n in range(4)]
        return [partial(piece, r) for r in range(0, D2 // 2, 48)]

    def stage_e(slot, z0, z1, r):
        def act(h):
            rr = pl.ds(pl.multiple_of(z0 + r + h, 8), 8)
            aq, uq, dq = (_sum7([big[i, rr, k * W2:(k + 1) * W2] for i in range(7)])
                          for k in range(3))
            out = []
            for n, (a, u, dm) in enumerate(zip(aq, uq, dq)):
                sg = 1.0 / (1.0 + jnp.exp(-a))
                g = a * sg
                for k, v in enumerate((dm * u * (sg + g * (1.0 - sg)), dm * g, g * u)):
                    out.append((big, (14, pl.ds(pl.multiple_of(z1 + n * 16 + h, 8), 8),
                                      slice(k * W2, (k + 1) * W2)), v))
            return out

        def pack(k):
            c = slice(k * W2, (k + 1) * W2)
            v = [big[14, rws(z0 + n * 16, 16), c] for n in range(4)]
            rr = pl.ds(pl.multiple_of(z1 + slot * (H2 // 2) + r // 2, 8), 8)
            return [(big, (7 + i, rr, c), pltpu.bitcast(o.astype(bf16), f32))
                    for i, o in enumerate(_rhs7(*v))]
        return [partial(act, 0), partial(act, 8)] + [partial(pack, k) for k in range(3)]

    def store(items):
        for ref, idx, v in items:
            ref[idx] = v

    def run(dots, pieces=()):
        n, done = sum(w for w, _ in dots), 0
        for w, dot in dots:
            lo, hi = len(pieces) * done // n, len(pieces) * (done + w) // n
            done += w
            dot()
            for piece in pieces[lo:hi]:
                store(piece())
        if not dots:
            for piece in pieces:
                store(piece())

    lo, hi = slice(0, 2 * W2), slice(2 * W2, 3 * W2)

    def stage_a(f, s_):
        def dot(i, src, c):
            big[i, :, c] = _nn(src[s_, i, :, 0:KS[i]], wB[f % 2, i, 0:KS[i], c])
        return [d for i in range(7)
                for d in ((2, partial(dot, i, hA, lo)), (1, partial(dot, i, dA, hi)))]

    def stage_b(f, s_):
        def p(i, c):
            return pltpu.bitcast(big[7 + i, rws(s_ * (H2 // 2), H2 // 2), c], bf16)

        def dx(i, acc, c):
            acc[s_, i] += _nt(wA[f % 3, i, :, c], p(i, c))

        def dw(i, src, c):
            gacc[f % 2, i, :, c] = (jnp.where(s_ == 0, 0.0, gacc[f % 2, i, :, c])
                                    + _nn(src[s_, i], p(i, c)))
        return [d for i in range(7) for d in (
            (2, partial(dx, i, accG, lo)), (1, partial(dx, i, accO, hi)),
            (2, partial(dw, i, hTA, lo)), (1, partial(dw, i, dTA, hi)))]

    def each(fn, *a):
        return [piece for k in range(3) for piece in fn(*a, k)]

    for f in range(2):
        for k in range(3):
            w_copy(k, f).wait()

    def first_prep(n):
        run((), each(prep, n // 2, n % 2, 0))
    loop(4, first_prep)
    for k in range(3):
        w_copy(k, 2).start()

    def first_a(s_):
        run(stage_a(0, s_))

        @pl.when(s_ == 0)
        def _():
            loop(H2 // 64, lambda r: run((), [pc for q in range(0, 64, 16)
                                              for pc in stage_e(0, 0, 0, r * 64 + q)]))
    loop(2, first_a)

    def ffn(j):
        f, s_ = j // 2, j % 2

        @pl.when(s_ == 0)
        def _():
            @pl.when(f + 2 < NF)
            def _():
                for k in range(3):
                    w_copy(k, f + 2).wait()

            @pl.when(f + 3 < NF)
            def _():
                for k in range(3):
                    w_copy(k, f + 3).start()

            @pl.when(f >= 2)
            def _():
                for k in range(3):
                    g_copy(k, f - 2).start()

        z0, z1 = zs[0], zs[1]
        run(stage_b(f, s_), [pc for r in range(0, H2, 16) for pc in stage_e(1 - s_, z0, z1, r)])

        @pl.when((s_ == 0) & (f >= 3))
        def _():
            for k in range(3):
                g_copy(k, f - 3).wait()

        @pl.when(f + 1 < NF)
        def _():
            z0, z1 = zs[2], zs[3]

            def chained(piece):
                items = piece()
                return items + [(tok, (pl.ds(pl.multiple_of(z1 + 8, 8), 8), slice(None)),
                                 pltpu.bitcast(items[-1][2][-16:], jnp.uint32))]
            run(stage_a(f + 1, s_),
                [partial(chained, pc)
                 for pc in each(prep, f + 2, s_, z0) + each(finish_w, f + 1, s_, z0)])

        @pl.when(f + 1 == NF)
        def _():
            run((), each(finish_w, NF - 2, s_, 0))
    loop(2 * NF, ffn)
    for k in range(3):
        g_copy(k, NF - 2).start()
        g_copy(k, NF - 3).wait()

    def finish_last(s_):
        run((), each(finish_w, NF - 1, s_, 0))
    loop(2, finish_last)
    for k in range(3):
        g_copy(k, NF - 1).start()

    def ln2_bwd(n):
        s_, c, c1, c2 = pair(n)
        oq = _sum7t([accO[s_, i, :, c] for i in range(7)])
        gq = _sum7t([accG[s_, i, :, c] for i in range(7)])
        for m, cc in enumerate((c1, c2)):
            oT[0, 0:D2, cc] = oq[m].astype(bf16)
            oT[0, D2:D, cc] = oq[2 + m].astype(bf16)
            dh = doT[:, cc].astype(f32) + _ln_bwd(
                hnT[:, cc].astype(f32), r2[:, cc], jnp.concatenate([gq[m], gq[2 + m]], axis=0))
            dhT[:, cc] = dh
            butterflies(dh, cc)
    loop(8, ln2_bwd)
    o_copy(0).start()

    def filt_b(t, gr, gi):
        wr, wi = weights(0, t), weights(1, t)
        xr, xi = xs[0, t], xs[1, t]
        for k, v in enumerate((gr * xr + gi * xi, gi * xr - gr * xi)):
            for l0, r, n in CLASSES:
                wp[k, t, pl.ds(l0, n, stride=9), :] = v[r:r + n]
            wp[k, t, DF - 1:LP, :] = v[DF - 1:LP]
        return gr * wr + gi * wi, gi * wr - gr * wi

    def dw_out(i):
        for k in range(2):
            rr = slice(DF - 1, LP) if i is None else rows(i)
            v = _to_natural_order([pltpu.bitcast(wp[k, t, rr, :].astype(bf16), jnp.uint32)
                                   for t in range(NT)])
            for t in range(NT):
                vb = pltpu.bitcast(v[t], bf16)
                if i is None:
                    dwv[k, DF - 1:DF, _tile(t)] = vb[0:1]
                else:
                    dwv[k, rr, _tile(t)] = vb
        if i is None:
            o_copy(1).start()
            o_copy(2).start()
    spectral(filt_b, side_last=dw_out)

    def ln1_bwd(n):
        for c in (cols(2 * n, 128), cols(2 * n + 1, 128)):
            dx = dhT[:, c] + _ln_bwd(xnT[:, c].astype(f32), r1[:, c], unbutterfly(c))
            oT[1, :, c] = dx.astype(bf16)
        dx_copy(n).start()
    loop(8, ln1_bwd)
    for n in range(8):
        dx_copy(n).wait()
    for f in (NF - 2, NF - 1):
        for k in range(3):
            g_copy(k, f).wait()
    for k in range(3):
        o_copy(k).wait()


@jax.jit
def pallas_sequential_preLN__spectral_gfnet__swiglu_ffn__prompt_kernel(
    A_x: jax.Array,
    A_w_r: jax.Array,
    A_w_i: jax.Array,
    B_x: jax.Array,
    B_w_gate: jax.Array,
    B_w_up: jax.Array,
    B_w_down: jax.Array,
    grad_out: jax.Array,
):
    sds = lambda shape: jax.ShapeDtypeStruct(shape, bf16)
    hbm = pl.BlockSpec(memory_space=pl.ANY)
    vm = pltpu.VMEM
    outT, dxT, dwrT, dwiT, dwg, dwu, dwdT = pl.pallas_call(
        _kernel,
        in_specs=[hbm] * 10,
        out_specs=[hbm] * 7,
        out_shape=[sds((D, S)), sds((D, S)), sds((DF, S)), sds((DF, S)),
                   sds((D, F)), sds((D, F)), sds((D, F))],
        scratch_shapes=[
            vm((D, S), bf16), vm((D, S), bf16), vm((2, DF, S), bf16),
            vm(_CD.shape, bf16), vm(_CI.shape, bf16), vm(_BS.shape, bf16),
            vm((3, 2, D, FT), bf16), vm((3, 2, D, FT), bf16),
            vm((2, D, S), bf16), vm((2, DF, S), bf16),
            vm((D, S), bf16), vm((1, S), f32),
            vm((D, S), bf16), vm((1, S), f32), vm((D, S), bf16), vm((D, S), f32),
            vm((2 * LP, S), f32), vm((NT, LP, 256), bf16),
            vm((2, NT, LP, 128), f32), vm((2, NT, LP, 128), f32),
            vm((D, S), f32), vm((15, H2, 3 * W2), f32), vm((16, 128), jnp.uint32), pltpu.SMEM((4,), jnp.int32),
            vm((2, 7, D2, H2), f32),
            vm((2, 7, D2, H2), f32), vm((2, 7, D2, 3 * W2), f32),
            vm((2, 7, H2, 320), bf16), vm((2, 7, H2, 320), bf16),
            vm((2, 7, D2, H2), bf16), vm((2, 7, D2, H2), bf16),
            vm((2, 7, 320, 3 * W2), bf16), vm((3, 7, D2, 3 * W2), bf16),
            pltpu.SemaphoreType.DMA((7,)), pltpu.SemaphoreType.DMA((3, 2)),
            pltpu.SemaphoreType.DMA((3, 2)), pltpu.SemaphoreType.DMA((11,)),
        ],
        compiler_params=pltpu.CompilerParams(vmem_limit_bytes=126 * 2**20),
    )(A_x[0].T, grad_out[0].T, A_w_r.T, A_w_i.T, _CD, _CI, _BS,
      B_w_gate, B_w_up, B_w_down.T)
    return (outT.T[None], dxT.T[None], dwrT.T, dwiT.T, dwg, dwu, dwdT.T)
```

```python
from functools import partial

import numpy as np
import jax
import jax.numpy as jnp
from jax import lax
import jax.experimental.pallas as pl
import jax.experimental.pallas.tpu as pltpu

S, D, F = 2048, 576, 4608
DF = D // 2 + 1
LP = 304
NT = S // 128
FT = 256
ST = 1024
H2, W2, D2 = ST // 2, FT // 2, D // 2
NF = F // FT
EPS = 1e-5
bf16, f32, u32 = jnp.bfloat16, jnp.float32, jnp.uint32


CLASSES = [(l0, 32 * n, 32) for n, l0 in enumerate((1, 8, 2, 7, 3, 6, 4, 5, 0))]
COS = tuple(float(np.cos(2 * np.pi * k / 9)) for k in (1, 2, 4)) + (1.0,)
SIN = tuple(float(np.sin(2 * np.pi * k / 9)) for k in (1, 2, 4)) + (-1.0,)
SIN3 = float(np.sin(2 * np.pi / 3))


def _consts():
    d2 = np.arange(64)[None, :]

    def block(l, sign):
        a = 2.0 * np.pi * ((l[:, None] * d2) % D) / D
        re = np.concatenate([np.cos(a), sign * np.sin(a)], axis=1)
        im = np.concatenate([-np.sin(a), sign * np.cos(a)], axis=1)
        return re, im
    cd = np.zeros((5, 128, 128))
    ms = np.full((5, 128), 2.0 / (S * D))
    for r in range(1, 5):
        (ra, ia), (rb, ib) = block(r + 9 * np.arange(32), -1), block(9 - r + 9 * np.arange(32), 1)
        cd[r - 1] = np.concatenate([ra, rb, ia, ib])
    r0, i0 = block(9 * np.arange(33), 0)
    cd[4, 0:33], cd[4, 49:80] = r0, i0[1:32]
    ms[4, 0] = ms[4, 32] = 1.0 / (S * D)
    ci = (cd * ms[:, :, None]).transpose(0, 2, 1)
    q = np.arange(128)
    s2 = np.arange(128)[:, None]
    bs = np.zeros((NT, 256, 256))
    for k1 in range(NT):
        tile = (q - k1) % 16
        k = 128 * tile + (q - tile) % 128
        a = 2.0 * np.pi * ((s2 * k[None, :]) % S) / S
        mr, mi = np.cos(a), -np.sin(a)
        bs[k1] = np.block([[mr, mi], [-mi, mr]])
    t = lambda v: np.asarray(v, np.float32).astype(bf16)
    return t(cd), t(ci), t(bs)


_CD, _CI, _BS = _consts()


def _nn(a, b):
    return lax.dot_general(a, b, (((1,), (0,)), ((), ())), preferred_element_type=f32)


def _nt(a, b):
    return lax.dot_general(a, b, (((1,), (1,)), ((), ())), preferred_element_type=f32)


def _tw(re, im, p, sign):
    p = p % 16
    if p == 0:
        return re, im
    if p == 4:
        return (-im, re) if sign > 0 else (im, -re)
    if p == 8:
        return -re, -im
    c = float(np.cos(2 * np.pi * p / 16))
    s = float(sign * np.sin(2 * np.pi * p / 16))
    if p % 2 == 0:
        q = s / c
        if q > 0:
            return (re - im) * c, (re + im) * c
        return (re + im) * c, (im - re) * c
    return re * c - im * s, re * s + im * c


def _fft4(v, sign):
    (ar, ai), (br, bi), (cr, ci), (dr, di) = v
    pr, pi_, qr, qi = ar + cr, ai + ci, ar - cr, ai - ci
    sr, si, tr, ti = br + dr, bi + di, br - dr, bi - di
    o1, o3 = (qr - ti, qi + tr), (qr + ti, qi - tr)
    if sign < 0:
        o1, o3 = o3, o1
    return [(pr + sr, pi_ + si), o1, (pr - sr, pi_ - si), o3]


def _fft16(v, sign):
    cols = [_fft4([v[4 * a + b] for a in range(4)], sign) for b in range(4)]
    out = [None] * 16
    for c in range(4):
        r = _fft4([_tw(*cols[b][c], b * c, sign) for b in range(4)], sign)
        for e in range(4):
            out[c + 4 * e] = r[e]
    return out


def _rot3(c, v):
    return [c[0] * v[0] + c[1] * v[1] + c[2] * v[2],
            c[1] * v[0] + c[2] * v[1] + (c[3] * c[0]) * v[2],
            c[2] * v[0] + (c[3] * c[0]) * v[1] + (c[3] * c[1]) * v[2]]


def _radix9(x):
    s1, s2, s3, s4 = (x[b] + x[9 - b] for b in range(1, 5))
    d1, d2, d3, d4 = (x[b] - x[9 - b] for b in range(1, 5))
    a, t, e, g = x[0] + s3, s1 + s2 + s4, x[0] - 0.5 * s3, SIN3 * d3
    r1, r2, r4 = _rot3(COS, (s1, s2, s4))
    p1, p2, p4 = _rot3(SIN, (d1, d2, d4))
    return [e + r1, p1 + g, e + r2, p2 - g, a - 0.5 * t, SIN3 * (d1 - d2 + d4),
            e + r4, p4 + g, a + t]


def _radix9_t(v):
    r1, p1, r2, p2, r3, p3, r4, p4, dc = v
    a, t, e, g = dc + r3, r1 + r2 + r4, dc - 0.5 * r3, SIN3 * p3
    s1, s2, s4 = _rot3(COS, (r1, r2, r4))
    d1, d2, d4 = _rot3(SIN, (p1, p2, p4))
    sm = [e + s1, e + s2, a - 0.5 * t, e + s4]
    df = [d1 + g, d2 - g, SIN3 * (p1 - p2 + p4), d4 + g]
    return [a + t] + [sm[b] + df[b] for b in range(4)] + [sm[b] - df[b] for b in (3, 2, 1, 0)]


def _barrel(t, sign):
    lane = lax.broadcasted_iota(jnp.int32, t[0].shape, 1)
    for i in range(4):
        hi = (lane & (1 << i)) != 0
        t = [jnp.where(hi, t[(p + sign * (1 << i)) % 16], t[p]) for p in range(16)]
    return t


def _to_spectral_order(t):
    r = [pltpu.roll(v, n, 1) if n else v for n, v in enumerate(t)]
    return _barrel([r[-m % 16] for m in range(16)], -1)


def _to_natural_order(t):
    r = _barrel(t, +1)
    return [pltpu.roll(r[-n % 16], 128 - n, 1) if n else r[0] for n in range(16)]


def _lhs7(a11, a12, a21, a22):
    return [a11 + a22, a21 + a22, a11, a22, a11 + a12, a21 - a11, a12 - a22]


def _rhs7(b11, b12, b21, b22):
    return [b11 + b22, b11, b12 - b22, b21 - b11, b22, b11 + b12, b21 + b22]


def _sum7(m):
    return (m[0] + m[3] - m[4] + m[6], m[2] + m[4], m[1] + m[3], m[0] - m[1] + m[2] + m[5])


def _lhs7t(a11, a12, a21, a22):
    return [a11 - a22, a21 - a22, a12 - a22, a11 - a21, a11 - a12, a22, a11]


def _sum7t(n):
    return (n[0] + n[5] - n[4] + n[2], n[6] - n[4], n[1] + n[5], n[1] - n[0] + n[6] - n[3])


def _tile(t):
    return slice(128 * t, 128 * (t + 1))


def _split(v):
    u = v if v.dtype == u32 else pltpu.bitcast(v, u32)
    return [pltpu.unpack_elementwise(u, index=e, packed_dtype=bf16, unpacked_dtype=f32)
            for e in (0, 1)]


def _join(even, odd):
    return pltpu.pack_elementwise([even, odd], packed_dtype=bf16)


def _combine(fn, blocks):
    parts = [_split(b) for b in blocks]
    return [_join(e, o) for e, o in zip(fn(*[q[0] for q in parts]), fn(*[q[1] for q in parts]))]


def _fold(acc, v):
    for r in range(0, v.shape[0], 8):
        acc = v[r:r + 8] if acc is None else acc + v[r:r + 8]
    return acc


def _mean(acc):
    return jnp.sum(acc, axis=0, keepdims=True) * (1.0 / D)


def _rows(n, stop, base=0):
    return [slice(base + r, base + r + n) for r in range(0, stop, n)]


def _rstd(get, mean):
    acc = None
    for rr in _rows(16, D):
        c = get(rr) - mean
        acc = _fold(acc, c * c)
    return lax.rsqrt(_mean(acc) + EPS)


def _kernel(xT_h, doT_h, wrT_h, wiT_h, cd_h, ci_h, bs_h, wg_h, wu_h, wdT_h,
            outT_h, dxT_h, dwrT_h, dwiT_h, dwg_h, dwu_h, dwdT_h,
            xT, doT, wv, cd, ci, bs, wts, gws, oT, dwv,
            xnT, r1, hnT, r2, ub, yv, z, zb, xs, wp, dhT, big, tok, zs, accO, accG, gacc,
            hA, dA, hTA, dTA, wB, wA, p0, p1,
            sem_in, sem_w, sem_g, sem_o):
    def cols(i, n):
        return pl.ds(pl.multiple_of(i * n, n), n)

    def in_copy(k):
        src, dst = ((xT_h, xT), (cd_h, cd), (wrT_h, wv.at[0]), (wiT_h, wv.at[1]),
                    (doT_h, doT), (bs_h, bs), (ci_h, ci))[k]
        return pltpu.make_async_copy(src, dst, sem_in.at[k])

    def w_copy(k, f):
        return pltpu.make_async_copy((wg_h, wu_h, wdT_h)[k].at[:, cols(f, FT)],
                                     wts.at[k, f % 2], sem_w.at[k, f % 2])

    def g_copy(k, f):
        return pltpu.make_async_copy(gws.at[k, f % 2], (dwg_h, dwu_h, dwdT_h)[k].at[:, cols(f, FT)],
                                     sem_g.at[k, f % 2])

    def o_copy(k):
        src, dst = ((oT.at[0], outT_h), (dwv.at[0], dwrT_h), (dwv.at[1], dwiT_h))[k]
        return pltpu.make_async_copy(src, dst, sem_o.at[k])

    def dx_copy(n):
        return pltpu.make_async_copy(oT.at[1, :, cols(n, 256)], dxT_h.at[:, cols(n, 256)],
                                     sem_o.at[3 + n])

    in_copy(0).start()
    in_copy(1).start()

    def loop(n, fn):
        lax.fori_loop(0, n, lambda i, c: (fn(i), c)[1], 0)

    def rws(start, n):
        return pl.ds(start if isinstance(start, int) else pl.multiple_of(start, 16), n)

    def rows(i):
        return cols(i, 16)

    def rows_im(i):
        return pl.ds(pl.multiple_of(LP + i * 16, 16), 16)

    def strided():
        return [[slice(64 * b + r, 64 * b + r + 16) for b in range(9)] for r in range(0, 64, 16)]

    def butterflies(get, c):
        for group in strided():
            for rr, v in zip(group, _radix9([get(rr) for rr in group])):
                ub[rr, c] = v.astype(bf16)

    def unbutterfly(c):
        for group in strided():
            yield from zip(group, _radix9_t([yv[rr, c] for rr in group]))

    def spectral(filt, extra, side=None, side_last=None):
        for r in range(4):
            v = _nn(cd[r], ub[128 * r:128 * (r + 1), :])
            z[64 * r:64 * (r + 1), :] = v[0:64]
            z[LP + 64 * r:LP + 64 * (r + 1), :] = v[64:128]
        v = _nn(cd[4, 0:96, 0:64], ub[512:576, :])
        z[256:LP, :] = v[0:48]
        z[LP + 256:2 * LP, :] = v[48:96]

        def fft16(i, sign):
            v = [(z[rows(i), _tile(t)], z[rows_im(i), _tile(t)]) for t in range(NT)]
            o = _fft16(v, sign)
            for t in range(NT):
                zb[t, rows(i), 0:128] = o[t][0].astype(bf16)
                zb[t, rows(i), 128:256] = o[t][1].astype(bf16)
        if side is None:
            loop(LP // 16, partial(fft16, sign=-1))
        else:
            in_copy(2).wait()
            in_copy(3).wait()
            loop(LP // 16 - 1, lambda i: (fft16(i, -1), side(i)))
            fft16(LP // 16 - 1, -1)
            side(None)

        def sstage(j):
            for t in [4 * j + n for n in range(4)]:
                v = _nn(zb[t], bs[t])
                yr, yi = filt(t, v[:, 0:128], v[:, 128:256])
                v = _nt(jnp.concatenate([yr, yi], axis=1).astype(bf16), bs[t])
                z[0:LP, cols(t, 128)] = v[:, 0:128]
                z[LP:2 * LP, cols(t, 128)] = v[:, 128:256]
            extra(2 * j)
            extra(2 * j + 1)
        loop(NT // 4, sstage)
        if side_last is None:
            loop(LP // 16, partial(fft16, sign=1))
        else:
            o_copy(0).start()
            loop(LP // 16 - 1, lambda i: (fft16(i, 1), side_last(i)))
            fft16(LP // 16 - 1, 1)
            side_last(None)

        def istage(j):
            for r, (a, b) in enumerate([(64 * n, 64 * n + 64) for n in range(4)] + [(256, LP)]):
                rhs = jnp.concatenate(
                    [jnp.concatenate([zb[4 * j + n, a:b, 0:128], zb[4 * j + n, a:b, 128:256]], axis=0)
                     for n in range(4)], axis=1)
                m = 128 if r < 4 else 64
                yv[128 * r:128 * r + m, cols(j, 512)] = _nn(ci[r, 0:m, 0:2 * (b - a)], rhs)
        loop(NT // 4, istage)

    def weights(k, t):
        return jnp.concatenate([wp[k, t, pl.ds(l0, n, stride=9), :] for l0, _, n in CLASSES]
                               + [wp[k, t, DF - 1:LP, :]], axis=0)

    def pair(n):
        s_, t = n // 4, n % 4
        return s_, cols(t, 128), cols(s_ * 8 + t, 128), cols(s_ * 8 + 4 + t, 128)

    def clear(n):
        s_, c, _, _ = pair(n)
        for i in range(7):
            accG[s_, i, :, c] = jnp.zeros((D2, 128), f32)
            if i in (0, 4, 5):
                accO[s_, i, :, c] = jnp.zeros((D2, 128), f32)
    loop(8, clear)

    def clear_dw(i):
        gacc[1, i] = jnp.zeros(gacc.shape[2:], f32)
    loop(7, clear_dw)
    in_copy(0).wait()
    for k in (2, 3, 5):
        in_copy(k).start()

    def ln1(c):
        x = lambda rr: xT[rr, c].astype(f32)
        acc = None
        for rr in _rows(16, D):
            acc = _fold(acc, x(rr))
        mean = _mean(acc)
        r = _rstd(x, mean)
        r1[:, c] = r

        def norm(rr):
            n = (x(rr) - mean) * r
            xnT[rr, c] = n.astype(bf16)
            return n
        butterflies(norm, c)
    loop(NT // 2, lambda n: (ln1(cols(2 * n, 128)), ln1(cols(2 * n + 1, 128))))
    in_copy(1).wait()
    in_copy(4).start()
    in_copy(6).start()
    for f in range(2):
        for k in range(3):
            w_copy(k, f).start()

    def wperm(i):
        for k in range(2):
            if i is None:
                last = jnp.broadcast_to(wv[k, DF - 1:DF, :].astype(f32), (16, S))
                first_row = lax.broadcasted_iota(jnp.int32, (16, S), 0) == 0
                v, rr = jnp.where(first_row, last, 0.0).astype(bf16), slice(DF - 1, LP)
            else:
                v, rr = wv[k, rows(i), :], rows(i)
            o = _to_spectral_order([pltpu.bitcast(v[:, _tile(t)], jnp.uint32) for t in range(NT)])
            for t in range(NT):
                wp[k, t, rr, :] = pltpu.bitcast(o[t], bf16).astype(f32)
        if i is None:
            in_copy(4).wait()
            in_copy(5).wait()
            in_copy(6).wait()

    def filt(t, xr, xi):
        row = lax.broadcasted_iota(jnp.int32, (LP, 128), 0)
        sc = jnp.where((row == 256) | (row == 288), 1.0 / (S * D), 2.0 / (S * D)).astype(f32)
        wr, wi = weights(0, t), weights(1, t)
        xs[0, t] = xr * sc
        xs[1, t] = xi * sc
        return xr * wr - xi * wi, xr * wi + xi * wr

    KS = (256, 256, 320, 320, 256, 320, 320)

    def operands(n, src, lhs, lhs_t):
        s_, c, c1, c2 = pair(n)
        for ra, rb in zip(_rows(48, D2), _rows(48, D2, D2)):
            blk = [src[rr, cc] for rr in (ra, rb) for cc in (c1, c2)]
            for i, o in enumerate(_combine(_lhs7, blk)):
                lhs_t[s_, i, ra.start // 2:ra.stop // 2, c] = o
        for d in (0, 128):
            blk = [src[dd:dd + 128, cc].T for cc in (c1, c2) for dd in (d, 256 + d)]
            for rr in _rows(16, 128):
                for i, o in enumerate(_lhs7(*[jnp.concatenate(_split(b[rr])) for b in blk])):
                    lhs[s_, i, rws(n % 4 * 128 + rr.start, 16), d:d + 128] = o.astype(bf16)
        ta, tb = src[512:, c1].T, src[512:, c2].T
        for rr in _rows(16, 128):
            t1, t2 = jnp.concatenate(_split(ta[rr])), jnp.concatenate(_split(tb[rr]))
            for i, o in ((2, t1), (3, t2), (5, t2 - t1), (6, t1 - t2)):
                lhs[s_, i, rws(n % 4 * 128 + rr.start, 16), 256:320] = o.astype(bf16)

    spectral(filt, lambda n: operands(n, doT, dA, dTA), side=wperm)

    def ln2(n):
        s_, c, c1, c2 = pair(n)
        for cc in (c1, c2):
            acc = None
            for rr, y in unbutterfly(cc):
                h = y + xT[rr, cc].astype(f32)
                dhT[rr, cc] = h
                acc = _fold(acc, h)
            mean = _mean(acc)
            r = _rstd(lambda rr: dhT[rr, cc], mean)
            r2[:, cc] = r
            for rr in _rows(32, D):
                hnT[rr, cc] = ((dhT[rr, cc] - mean) * r).astype(bf16)
        for ra, rb in zip(_rows(48, D2), _rows(48, D2, D2)):
            h11, h12, h21, h22 = (dhT[rr, cc] for rr in (ra, rb) for cc in (c1, c2))
            for i, o in ((2, h11), (6, h12), (1, h21), (3, h12 + h21 - h22)):
                accO[s_, i, ra, c] = o
        operands(n, hnT, hA, hTA)
    loop(8, ln2)

    tok[...] = jnp.zeros_like(tok)
    big[7, 72:80, 0:128] = jnp.zeros((8, 128), f32)
    for n in range(4):
        zs[n] = 0

    def gated(v, gate):
        u = pltpu.bitcast(v, u32)
        if gate is None:
            return u
        return u | jnp.tile(gate(), (u.shape[0] // 8, u.shape[1] // 128))

    def words(start, n):
        return pl.ds(pl.multiple_of(start // 2, 8), n // 2)

    def prep(f, half, forward, gate, k):
        c = slice(k * W2, (k + 1) * W2)

        def blocks(r0, r1_, n):
            top = gated(wts[k, f % 2, rws(r0, n), :], gate)
            bot = gated(wts[k, f % 2, rws(r1_, n), :], gate)
            return top[:, :W2], top[:, W2:], bot[:, :W2], bot[:, W2:]

        def fwd(r):
            r = half * 128 + r
            return [(wB, (f % 3, i, words(r, 32), c), o)
                    for i, o in enumerate(_combine(_rhs7, blocks(r, 256 + r, 32)))]

        def tail():
            v = gated(wts[k, f % 2, rws(512 + half * 32, 32), :], gate)
            return [(wB, (f % 3, i, words(256 + half * 32, 32), c), v[:, n * W2:(n + 1) * W2])
                    for i, n in ((2, 1), (3, 0), (5, 1), (6, 0))]

        def bwd(r):
            r = half * (D2 // 2) + r
            return [(wA, (f % 3, i, words(r, 48), c), o)
                    for i, o in enumerate(_combine(_lhs7t, blocks(r, D2 + r, 48)))]
        if forward:
            return [partial(fwd, r) for r in range(0, 128, 32)] + [tail]
        return [partial(bwd, r) for r in range(0, D2 // 2, 48)]

    def finish_w(f, half, gate, k):
        def piece(r):
            r = half * (D2 // 2) + r
            cq = _sum7([pltpu.bitcast(gated(gacc[f % 2, i, rws(r, 48), k * W2:(k + 1) * W2], gate), f32)
                        for i in range(7)])
            return [(gws, (k, f % 2, rws((n // 2) * D2 + r, 48),
                           slice((n % 2) * W2, (n % 2 + 1) * W2)), cq[n].astype(bf16))
                    for n in range(4)]
        return [partial(piece, r) for r in range(0, D2 // 2, 48)]

    def link(z1, v):
        return big, (7, pl.ds(pl.multiple_of(z1 + 64, 8), 8), slice(0, 128)), pltpu.bitcast(v, f32)

    def stage_e(dst, z0, z1, r):
        def act(h):
            rr = pl.ds(pl.multiple_of(z0 + r + h, 8), 8)
            aq, uq, dq = (_sum7([big[i, rr, k * W2:(k + 1) * W2] for i in range(7)])
                          for k in range(3))
            out = []
            for n, (a, u, dm) in enumerate(zip(aq, uq, dq)):
                sg = 1.0 / (1.0 + jnp.exp(-a))
                g = a * sg
                for k, v in enumerate((dm * u * (sg + g * (1.0 - sg)), dm * g, g * u)):
                    out.append((big, (7, pl.ds(pl.multiple_of(z1 + n * 16 + h, 8), 8),
                                      slice(k * W2, (k + 1) * W2)), v))
            return out

        def pack(k):
            c = slice(k * W2, (k + 1) * W2)
            ev, od = (_rhs7(*[big[7, pl.ds(pl.multiple_of(z0 + n * 16 + h, 8), 8), c]
                              for n in range(4)]) for h in (0, 8))
            out = [_join(e, o) for e, o in zip(ev, od)]
            return [(dst, (i, words(r, 16), c), o) for i, o in enumerate(out)] + [link(z1, out[-1])]
        return [partial(act, 0), partial(act, 8)] + [partial(pack, k) for k in range(3)]

    def store(items):
        for ref, idx, v in items:
            ref[idx] = v

    def run(dots, pieces=()):
        n, done = sum(w for w, _ in dots), 0
        for w, dot in dots:
            lo, hi = len(pieces) * done // n, len(pieces) * (done + w) // n
            done += w
            dot()
            for piece in pieces[lo:hi]:
                store(piece())
        if not dots:
            for piece in pieces:
                store(piece())

    lo, hi = slice(0, 2 * W2), slice(2 * W2, 3 * W2)

    def stage_a(f, s_):
        def dot(i, src, c):
            big[i, :, c] = _nn(src[s_, i, :, 0:KS[i]], pltpu.bitcast(wB[f % 3, i, 0:KS[i] // 2, c], bf16))
        return [d for i in range(7)
                for d in ((2, partial(dot, i, hA, lo)), (1, partial(dot, i, dA, hi)))]

    def stage_b(f, s_):
        def p(i, c):
            return pltpu.bitcast((p0, p1)[s_][i, :, c], bf16)

        def dx(i, acc, c):
            acc[s_, i] += _nt(pltpu.bitcast(wA[f % 3, i, :, c], bf16), p(i, c))

        def dw(i, src, c):
            v = _nn(pltpu.bitcast(src[s_, i], bf16), p(i, c))
            gacc[f % 2, i, :, c] = gacc[f % 2, i, :, c] + v if s_ else v
        return [d for i in range(7) for d in (
            (2, partial(dx, i, accG, lo)), (1, partial(dx, i, accO, hi)),
            (2, partial(dw, i, hTA, lo)), (1, partial(dw, i, dTA, hi)))]

    def each(fn, *a):
        return [piece for k in range(3) for piece in fn(*a, k)]

    for f in range(2):
        for k in range(3):
            w_copy(k, f).wait()

    def first_prep(n):
        run((), each(prep, n // 2, n % 2, True, None) + each(prep, n // 2, n % 2, False, None))
    loop(4, first_prep)
    for k in range(3):
        w_copy(k, 2).start()

    def first_a(s_):
        run(stage_a(0, s_))

        @pl.when(s_ == 0)
        def _():
            loop(H2 // 64, lambda r: run((), [pc for q in range(0, 64, 16)
                                              for pc in stage_e(p0, 0, 0, r * 64 + q)]))
    loop(2, first_a)

    def step(f, s_):
        z0, z1 = zs[0], zs[1]

        def linked(piece):
            items = piece()
            return items + [link(z1, items[-1][2][-8:])]
        gate = lambda: pltpu.bitcast(big[7, pl.ds(pl.multiple_of(z0 + 72, 8), 8), 0:128], u32)
        run(stage_b(f, s_),
            [pc for r in range(0, H2, 16) for pc in stage_e((p1, p0)[s_], z0, z1, r)]
            + [partial(linked, pc) for pc in each(prep, f + 2, s_, True, gate)])

        @pl.when(f + 1 < NF)
        def _():
            z0, z1 = zs[2], zs[3]

            def linked(piece):
                items = piece()
                return items + [(tok, (pl.ds(pl.multiple_of(z1 + 8, 8), 8), slice(None)),
                                 pltpu.bitcast(items[-1][2], u32)[-8:])]
            gate = lambda: tok[pl.ds(pl.multiple_of(z0, 8), 8), :]
            run(stage_a(f + 1, s_),
                [partial(linked, pc)
                 for pc in each(prep, f + 2, s_, False, gate) + each(finish_w, f + 1, s_, gate)])

    def ffn(f):
        @pl.when(f + 2 < NF)
        def _():
            for k in range(3):
                w_copy(k, f + 2).wait()

        @pl.when(f + 3 < NF)
        def _():
            for k in range(3):
                w_copy(k, f + 3).start()

        @pl.when(f >= 2)
        def _():
            for k in range(3):
                g_copy(k, f - 2).start()

        @pl.when(f >= 3)
        def _():
            for k in range(3):
                g_copy(k, f - 3).wait()
        step(f, 0)
        step(f, 1)
    loop(NF, ffn)
    loop(2, lambda s_: run((), each(finish_w, NF - 2, s_, None)))
    for k in range(3):
        g_copy(k, NF - 2).start()
        g_copy(k, NF - 3).wait()

    def finish_last(s_):
        run((), each(finish_w, NF - 1, s_, None))
    loop(2, finish_last)
    for k in range(3):
        g_copy(k, NF - 1).start()

    def ln2_bwd(n):
        s_, c, c1, c2 = pair(n)
        sums = [None] * 4
        for ra, rb in zip(_rows(16, D2), _rows(16, D2, D2)):
            gq = _sum7t([accG[s_, i, ra, c] for i in range(7)])
            for q, (rr, cc) in enumerate(((ra, c1), (ra, c2), (rb, c1), (rb, c2))):
                yv[rr, cc] = gq[q]
                sums[q % 2] = _fold(sums[q % 2], gq[q])
                sums[2 + q % 2] = _fold(sums[2 + q % 2], gq[q] * hnT[rr, cc].astype(f32))
        for m, cc in enumerate((c1, c2)):
            ma, mb, r = _mean(sums[m]), _mean(sums[2 + m]), r2[:, cc]

            def dh(rr):
                v = doT[rr, cc].astype(f32) + r * (yv[rr, cc] - ma - hnT[rr, cc].astype(f32) * mb)
                dhT[rr, cc] = v
                return v
            butterflies(dh, cc)
    loop(8, ln2_bwd)

    def out(n):
        s_, c, c1, c2 = pair(n)
        for ra, rb in zip(_rows(16, D2), _rows(16, D2, D2)):
            oq = _sum7t([accO[s_, i, ra, c] for i in range(7)])
            for v, (rr, cc) in zip(oq, ((ra, c1), (ra, c2), (rb, c1), (rb, c2))):
                oT[0, rr, cc] = v.astype(bf16)

    def filt_b(t, gr, gi):
        wr, wi = weights(0, t), weights(1, t)
        xr, xi = xs[0, t], xs[1, t]
        for k, v in enumerate((gr * xr + gi * xi, gi * xr - gr * xi)):
            for l0, r, n in CLASSES:
                wp[k, t, pl.ds(l0, n, stride=9), :] = v[r:r + n]
            wp[k, t, DF - 1:LP, :] = v[DF - 1:LP]
        return gr * wr + gi * wi, gi * wr - gr * wi

    def dw_out(i):
        for k in range(2):
            rr = slice(DF - 1, LP) if i is None else rows(i)
            v = _to_natural_order([pltpu.bitcast(wp[k, t, rr, :].astype(bf16), jnp.uint32)
                                   for t in range(NT)])
            for t in range(NT):
                vb = pltpu.bitcast(v[t], bf16)
                if i is None:
                    dwv[k, DF - 1:DF, _tile(t)] = vb[0:1]
                else:
                    dwv[k, rr, _tile(t)] = vb
        if i is None:
            o_copy(1).start()
            o_copy(2).start()
    spectral(filt_b, out, side_last=dw_out)

    def ln1_bwd(n):
        for c in (cols(2 * n, 128), cols(2 * n + 1, 128)):
            sa = sb = None
            for rr, g in unbutterfly(c):
                yv[rr, c] = g
                sa, sb = _fold(sa, g), _fold(sb, g * xnT[rr, c].astype(f32))
            ma, mb, r = _mean(sa), _mean(sb), r1[:, c]
            for rr in _rows(32, D):
                dx = dhT[rr, c] + r * (yv[rr, c] - ma - xnT[rr, c].astype(f32) * mb)
                oT[1, rr, c] = dx.astype(bf16)
        dx_copy(n).start()
    loop(8, ln1_bwd)
    for n in range(8):
        dx_copy(n).wait()
    for f in (NF - 2, NF - 1):
        for k in range(3):
            g_copy(k, f).wait()
    for k in range(3):
        o_copy(k).wait()


@jax.jit
def pallas_sequential_preLN__spectral_gfnet__swiglu_ffn__prompt_kernel(
    A_x: jax.Array,
    A_w_r: jax.Array,
    A_w_i: jax.Array,
    B_x: jax.Array,
    B_w_gate: jax.Array,
    B_w_up: jax.Array,
    B_w_down: jax.Array,
    grad_out: jax.Array,
):
    sds = lambda shape: jax.ShapeDtypeStruct(shape, bf16)
    hbm = pl.BlockSpec(memory_space=pl.ANY)
    vm = pltpu.VMEM
    outT, dxT, dwrT, dwiT, dwg, dwu, dwdT = pl.pallas_call(
        _kernel,
        in_specs=[hbm] * 10,
        out_specs=[hbm] * 7,
        out_shape=[sds((D, S)), sds((D, S)), sds((DF, S)), sds((DF, S)),
                   sds((D, F)), sds((D, F)), sds((D, F))],
        scratch_shapes=[
            vm((D, S), bf16), vm((D, S), bf16), vm((2, DF, S), bf16),
            vm(_CD.shape, bf16), vm(_CI.shape, bf16), vm(_BS.shape, bf16),
            vm((3, 2, D, FT), bf16), vm((3, 2, D, FT), bf16),
            vm((2, D, S), bf16), vm((2, DF, S), bf16),
            vm((D, S), bf16), vm((1, S), f32),
            vm((D, S), bf16), vm((1, S), f32), vm((D, S), bf16), vm((D, S), f32),
            vm((2 * LP, S), f32), vm((NT, LP, 256), bf16),
            vm((2, NT, LP, 128), f32), vm((2, NT, LP, 128), f32),
            vm((D, S), f32), vm((8, H2, 3 * W2), f32), vm((16, 128), jnp.uint32), pltpu.SMEM((4,), jnp.int32),
            vm((2, 7, D2, H2), f32),
            vm((2, 7, D2, H2), f32), vm((2, 7, D2, 3 * W2), f32),
            vm((2, 7, H2, 320), bf16), vm((2, 7, H2, 320), bf16),
            vm((2, 7, D2 // 2, H2), u32), vm((2, 7, D2 // 2, H2), u32),
            vm((3, 7, 160, 3 * W2), u32), vm((3, 7, D2 // 2, 3 * W2), u32),
            vm((7, H2 // 2, 3 * W2), u32), vm((7, H2 // 2, 3 * W2), u32),
            pltpu.SemaphoreType.DMA((7,)), pltpu.SemaphoreType.DMA((3, 2)),
            pltpu.SemaphoreType.DMA((3, 2)), pltpu.SemaphoreType.DMA((11,)),
        ],
        compiler_params=pltpu.CompilerParams(vmem_limit_bytes=126 * 2**20),
    )(A_x[0].T, grad_out[0].T, A_w_r.T, A_w_i.T, _CD, _CI, _BS,
      B_w_gate, B_w_up, B_w_down.T)
    return (outT.T[None], dxT.T[None], dwrT.T, dwiT.T, dwg, dwu, dwdT.T)
```
